```python
import jax
import jax.numpy as jnp

def _softmax(x, axis=-1):
    return jax.nn.softmax(x, axis=axis)
def _gelu(x):
    return jax.nn.gelu(x, approximate=True)
def _silu(x):
    return jax.nn.silu(x)
def _sigmoid(x):
    return jax.nn.sigmoid(x)
def _layernorm(x, axis=-1, eps=1e-5):
    m = jnp.mean(x, axis=axis, keepdims=True)
    v = jnp.var(x, axis=axis, keepdims=True)
    return (x - m) / jnp.sqrt(v + eps)
def _scatter_add(tgt, idx, src, axis=0):
    return tgt.at[idx].add(src)
def _segment_sum(src, seg, n):
    return jax.ops.segment_sum(src, seg, n)
class _Rng:
    def __init__(self, key):
        self._k = key
    def _next(self):
        self._k, sub = jax.random.split(self._k)
        return sub
    def normal(self, shape):
        return jax.random.normal(self._next(), shape, dtype=jnp.bfloat16)
    def randint(self, lo, hi, shape):
        return jax.random.randint(self._next(), shape, lo, hi, dtype=jnp.int32)
    def uniform(self, shape, lo=0.0, hi=1.0):
        return jax.random.uniform(self._next(), shape, jnp.bfloat16, lo, hi)
    def permutation(self, n):
        return jax.random.permutation(self._next(), n)


kernel_name = 'sequential_preLN__sliding_block_cached__glu_gated_swiglu__decode'

def setup_inputs():
    _rng = _Rng(jax.random.key(int.from_bytes(__import__("os").urandom(4), "little")))
    _w = (lambda a: (lambda t: t.astype(jnp.bfloat16) if jnp.issubdtype(t.dtype, jnp.floating) else t)(jnp.asarray(a)))
    def _A_setup():
        B, Sq, D = 1, 1, 640
        Hq, Hkv, Sk, Dh = 32, 32, 32768, 192
        assert Hq % Hkv == 0, (Hq, Hkv)
        return {
            "x": _w((lambda *s: _rng.normal(s) * 0.05)(B, Sq, D)),
            "k_cache": _w((lambda *s: _rng.normal(s) * 0.05)(B, Hkv, Sk, Dh)),
            "v_cache": _w((lambda *s: _rng.normal(s) * 0.05)(B, Hkv, Sk, Dh)),
            "wq": _w((lambda *s: _rng.normal(s) * 0.05)(D, Hq * Dh) * (D ** -0.5)),
            "wo": _w((lambda *s: _rng.normal(s) * 0.05)(Hq * Dh, D) * ((Hq * Dh) ** -0.5)),
        }
    _A_in = _A_setup()

    def _B_setup():
        B, S, D, F = 1, 1, 640, 1536
        return {
            "x": _w((lambda *s: _rng.normal(s) * 0.05)(B, S, D)),
            "w1": _w((lambda *s: _rng.normal(s) * 0.05)(D, F) * (2.0 / D) ** 0.5),
            "w3": _w((lambda *s: _rng.normal(s) * 0.05)(D, F) * (2.0 / D) ** 0.5),
            "w2": _w((lambda *s: _rng.normal(s) * 0.05)(F, D) * (2.0 / F) ** 0.5),
        }
    _B_in = _B_setup()

    return {
        "A_x": _A_in["x"],
        "A_k_cache": _A_in["k_cache"],
        "A_v_cache": _A_in["v_cache"],
        "A_wq": _A_in["wq"],
        "A_wo": _A_in["wo"],
        "B_x": _B_in["x"],
        "B_w1": _B_in["w1"],
        "B_w3": _B_in["w3"],
        "B_w2": _B_in["w2"],
    }

def reference(A_x, A_k_cache, A_v_cache, A_wq, A_wo, B_x, B_w1, B_w3, B_w2):
    def _A_ref(x, k_cache, v_cache, wq, wo):
        B, Sq, D = x.shape
        Hq, Dh = 32, 192
        Hkv, Sk = k_cache.shape[1], k_cache.shape[2]
        W = min(4096, max(256, Sk // 4))
        rep = Hq // Hkv
        q = (lambda x, *d: x.transpose(*d))((x @ wq).reshape(B, Sq, Hq, Dh), 0, 2, 1, 3)
        k = jnp.repeat(k_cache[:, :, Sk - W:, :], rep, axis=1)
        v = jnp.repeat(v_cache[:, :, Sk - W:, :], rep, axis=1)
        scores = jnp.einsum("bhqd,bhkd->bhqk", q, k) * (Dh ** -0.5)
        p = _softmax(scores, axis=-1)
        o = jnp.einsum("bhqk,bhkd->bhqd", p, v)
        return (lambda x, *d: x.transpose(*d))(o, 0, 2, 1, 3).reshape(B, Sq, Hq * Dh) @ wo

    def _B_ref(x, w1, w3, w2):
        gate = jnp.einsum("bsd,df->bsf", x, w1)
        up = jnp.einsum("bsd,df->bsf", x, w3)
        h = _silu(gate) * up
        out = jnp.einsum("bsf,fd->bsd", h, w2)
        return out

    x = A_x
    h = x + _A_ref(_layernorm(x, axis=-1), A_k_cache, A_v_cache, A_wq, A_wo)
    h2 = h + _B_ref(_layernorm(h, axis=-1), B_w1, B_w3, B_w2)
    return h2
```

```python
import jax
import jax.numpy as jnp
import numpy as np
from jax import lax
import jax.experimental.pallas as pl
import jax.experimental.pallas.tpu as pltpu

H, DH, SK, D, F = 32, 192, 32768, 640, 1536
W = min(4096, max(256, SK // 4))
BF = jnp.bfloat16
F32 = jnp.float32


def _bf16_round(v):
    u = int(np.float32(v).view(np.uint32))
    u = (u + 0x7FFF + ((u >> 16) & 1)) & 0xFFFF0000
    return float(np.uint32(u).view(np.float32))


SCALE = _bf16_round(DH ** -0.5)
EPS = _bf16_round(1e-5)


def _r(x):
    return x.astype(BF).astype(F32)


def _layernorm(x32):
    m = jnp.mean(x32, axis=-1, keepdims=True)
    c = x32 - m
    v = jnp.mean(c * c, axis=-1, keepdims=True)
    num = _r(x32 - _r(m))
    den = _r(jnp.sqrt(_r(_r(v) + EPS)))
    return (num / den).astype(BF)


def _blocks(rows, cols, phase, max_tiles, block, cuts=()):
    tr, n = cols // 128, rows // 8 * (cols // 128)
    edges = sorted({0, n} | set(range((-phase) % block, n, block)) | {c // 8 * tr for c in cuts})
    out = []
    for lo, hi in zip(edges[:-1], edges[1:]):
        segs = []
        while lo < hi:
            r, c = divmod(lo, tr)
            if c == 0 and hi - lo >= tr and tr <= max_tiles:
                nr = (hi - lo) // tr
                k = -(-nr // (max_tiles // tr))
                segs += [(r + i * nr // k, (i + 1) * nr // k - i * nr // k, 0, tr) for i in range(k)]
                lo += nr * tr
            else:
                nc = min(hi - lo, tr - c)
                k = -(-nc // max_tiles)
                segs += [(r, 1, c + i * nc // k, (i + 1) * nc // k - i * nc // k) for i in range(k)]
                lo += nc
        out.append([(8 * r, 8 * nr, 128 * c, 128 * nc) for r, nr, c, nc in segs])
    return out


def _scatter(blocks, stride):
    return [p for o in range(stride) for blk in blocks[o::stride] for p in blk]


def _window(spec):
    out = []
    for c0, n, widths, stride in spec:
        for r in _scatter([[r] for r in range(0, DH, 8 * n)], stride):
            out += [(r, min(8 * n, DH - r), 128 * (c0 + sum(widths[:i])), 128 * widths[i]) for i in range(len(widths))]
    return out


def _two_threads(tag0, pieces0, tag1, pieces1):
    items = []
    for t, (tag, pieces) in enumerate(((tag0, pieces0), (tag1, pieces1))):
        total, pos = sum(p[1] * p[3] for p in pieces), 0
        for p in pieces:
            items.append((pos / total, t, tag, p))
            pos += p[1] * p[3]
    return [(tag, p, t) for _, t, tag, p in sorted(items, key=lambda z: z[:2])]


def _halves(tag, blocks, stride):
    h = max(1, len(blocks) // 2)
    return _two_threads(tag, _scatter(blocks[:h], stride), tag, _scatter(blocks[h:], stride))


def _split(lst, n):
    return [lst[i * len(lst) // n:(i + 1) * len(lst) // n] for i in range(n)]


KV_BANDS = tuple((c, 5, (4,), 1) for c in range(0, W // 128, 4))


def make_kernel(R=3, kp=KV_BANDS, vp=KV_BANDS, wq=(0, 8, 8, 64), wo=(0, 8, 8, 64), pair=True,
                w13=(0, 8, 8, 32), w2=(0, 20, 20, 1), nq=4, n0=20, DA=384,
                w2ch=(512, 384, 384, 256), w2at=(0, 2, 4), vrot=0):
    N2 = len(w2ch)
    w2off = [sum(w2ch[:i]) for i in range(N2)]
    vp = _window(vp)
    kvp = _two_threads(0, _window(kp), 1, vp[vrot:] + vp[:vrot])
    NF = R - 1 + sum(max(0, w2at[c + 1] - w2at[c] - 1) for c in range(2))
    bq = _blocks(D, H * DH, *wq[:3])
    bo = [b for b in _blocks(H * DH, D, *wo[:3], cuts=(8 * NF,)) if b[0][0] >= 8 * NF]
    if pair:
        pro = _two_threads(0, _scatter(bq, wq[3]), 1, _scatter(bo, wo[3]))
    else:
        pro = _halves(0, bq, wq[3]) + _halves(1, bo, wo[3])
    b13 = _blocks(D, F, *w13[:3], cuts=(DA,))
    p13 = [_scatter([b for b in b13 if (b[0][0] >= DA) == c], w13[3]) for c in range(2)]
    w13p = [_two_threads(0, p, 1, p) for p in p13]
    b2 = _blocks(F, D, *w2[:3], cuts=w2off)
    w2p = [_halves(c, [b for b in b2 if w2off[c] <= b[0][0] < w2off[c] + w2ch[c]], w2[3]) for c in range(N2)]
    def kernel(x_hbm, kt_hbm, vt_hbm, wq_hbm, wo_hbm, w1_hbm, w3_hbm, w2_hbm, o_hbm,
               kv_v, wq_v, wo_v, w13_v, w2_v, q_v, x_v, o_v, sem_o):

        def body(sem_f, sem_w, sem_kv, sem_w13, sem_w2):
            def copy(job):
                src, dst, sem, p, _ = job
                idx = (pl.ds(p[0], p[1]), pl.ds(p[2], p[3]))
                return pltpu.make_async_copy(src.at[idx], dst.at[idx], sem)

            def issue(jobs):
                for j in jobs:
                    copy(j).start(priority=j[4])

            def wait_all(ref, sem):
                pltpu.make_async_copy(ref, ref, sem).wait()

            def head_jobs(h, slot):
                srcs = (kt_hbm.at[h, :, pl.ds(SK - W, W)], vt_hbm.at[h, :, pl.ds(SK - W, W)])
                return [(srcs[a], kv_v.at[slot, a], sem_kv.at[slot], p, t) for a, p, t in kvp]

            x_copy = pltpu.make_async_copy(x_hbm, x_v, sem_f.at[0])
            x_copy.start()
            jobs = [(wo_hbm, wo_v, sem_f.at[1 + i], (8 * i, 8, 0, D), (1 + i) % 2) for i in range(NF)]
            fences = [x_copy] + [copy(j) for j in jobs]
            issue(jobs + [((wq_hbm, wo_hbm)[a], (wq_v, wo_v)[a], sem_w, p, t) for a, p, t in pro])
            for h in range(R):
                fences.pop(0).wait()
                jobs = head_jobs(h, h)
                issue(jobs if h < R - 1 else jobs[:n0])
            wait_all(wq_v, sem_w)
            wait_all(wo_v.at[pl.ds(8 * NF, H * DH - 8 * NF)], sem_w)
            x32 = x_v[...].astype(F32)
            lnx = jnp.broadcast_to(_layernorm(x32), (8, D))
            QC = H // nq
            for c, group in enumerate(_split(jobs[n0:], nq)):
                qc = jnp.dot(lnx, wq_v[:, c * QC * DH:(c + 1) * QC * DH], preferred_element_type=F32)
                for j in range(QC):
                    q_v[c * QC + j] = qc[:, j * DH:(j + 1) * DH]
                issue(group)

            def head_compute(h, slot, attn):
                wait_all(kv_v.at[slot], sem_kv.at[slot])
                qh = q_v[h].astype(BF)
                s = jnp.dot(qh, kv_v[slot, 0], preferred_element_type=F32)
                s = _r(_r(s) * SCALE)
                m = jnp.max(s, axis=-1, keepdims=True)
                e = _r(jnp.exp(_r(s - m)))
                l = _r(jnp.sum(e, axis=-1, keepdims=True))
                p = (e / l).astype(BF)
                o = lax.dot_general(p, kv_v[slot, 1], (((1,), (1,)), ((), ())),
                                    preferred_element_type=F32)
                row = h * DH
                if not isinstance(h, int):
                    row = pl.multiple_of(row, DH)
                return attn + jnp.dot(o.astype(BF), wo_v[pl.ds(row, DH), :], preferred_element_type=F32)

            def head(h, attn):
                slot = h % R
                attn = head_compute(h, slot, attn)
                issue(head_jobs(h + R, slot))
                return attn

            attn = lax.fori_loop(0, H - R, head, jnp.zeros((8, D), F32))

            w13j = [[((w1_hbm, w3_hbm)[a], w13_v.at[a], sem_w13.at[c], p, t) for a, p, t in w13p[c]] for c in range(2)]
            w2j = [[(w2_hbm, w2_v, sem_w2.at[c], p, t) for _, p, t in w2p[c]] for c in range(N2)]
            for h, group in zip(range(H - R, H), _split(w13j[0], R - 1) + [w13j[1]]):
                attn = head_compute(h, h % R, attn)
                issue(group)
            hres = _r(x32 + _r(attn))
            lnh = _layernorm(hres)
            gate = up = 0.0
            for c, (r0, r1) in enumerate(((0, DA), (DA, D))):
                wait_all(w13_v.at[:, pl.ds(r0, r1 - r0)], sem_w13.at[c])
                gate = gate + jnp.dot(lnh[:, r0:r1], w13_v[0, r0:r1, :], preferred_element_type=F32)
                up = up + jnp.dot(lnh[:, r0:r1], w13_v[1, r0:r1, :], preferred_element_type=F32)
                for k in range(w2at[c], w2at[c + 1]):
                    if k > w2at[c]:
                        fences.pop(0).wait()
                    issue(w2j[k])
            assert not fences
            gate, up = _r(gate), _r(up)
            hm = (_r(gate * _r(jax.nn.sigmoid(gate))) * up).astype(BF)
            out = None
            for c in range(N2):
                r0, nr = w2off[c], w2ch[c]
                wait_all(w2_v.at[pl.ds(r0, nr)], sem_w2.at[c])
                o_ = jnp.dot(hm[:, r0:r0 + nr], w2_v[r0:r0 + nr, :], preferred_element_type=F32)
                out = o_ if out is None else out + o_
                if w2at[2] + c < N2:
                    issue(w2j[w2at[2] + c])
            res = hres + _r(out)
            o_v[...] = res[0:1, :].astype(o_v.dtype)
            pltpu.make_async_copy(o_v, o_hbm, sem_o).start()

        dma = pltpu.SemaphoreType.DMA
        pl.run_scoped(body, dma((1 + NF,)), dma(()), dma((R,)), dma((2,)), dma((N2,)))
        pltpu.make_async_copy(o_v, o_hbm, sem_o).wait()

    @jax.jit
    def run(A_x, A_k_cache, A_v_cache, A_wq, A_wo, B_x, B_w1, B_w3, B_w2):
        del B_x
        x = A_x.reshape(1, D)
        kt = jnp.swapaxes(A_k_cache.reshape(H, SK, DH), 1, 2)
        vt = jnp.swapaxes(A_v_cache.reshape(H, SK, DH), 1, 2)
        out = pl.pallas_call(
            kernel,
            out_shape=jax.ShapeDtypeStruct((1, D), A_x.dtype),
            in_specs=[pl.BlockSpec(memory_space=pl.ANY)] * 8,
            out_specs=pl.BlockSpec(memory_space=pl.ANY),
            scratch_shapes=[
                pltpu.VMEM((R, 2, DH, W), BF),
                pltpu.VMEM((D, H * DH), BF),
                pltpu.VMEM((H * DH, D), BF),
                pltpu.VMEM((2, D, F), BF),
                pltpu.VMEM((F, D), BF),
                pltpu.VMEM((H, 8, DH), F32),
                pltpu.VMEM((1, D), BF),
                pltpu.VMEM((1, D), BF),
                pltpu.SemaphoreType.DMA(()),
            ],
            compiler_params=pltpu.CompilerParams(vmem_limit_bytes=64 * 1024 * 1024),
        )(x, kt, vt, A_wq, A_wo, B_w1, B_w3, B_w2)
        return out.reshape(1, 1, D)

    return run


pallas_sequential_preLN__sliding_block_cached__glu_gated_swiglu__decode_kernel = make_kernel()
```

```python
import math

import jax
import jax.numpy as jnp
import numpy as np
from jax import lax
import jax.experimental.pallas as pl
import jax.experimental.pallas.tpu as pltpu

H, DH, SK, D, F = 32, 192, 32768, 640, 1536
W = min(4096, max(256, SK // 4))
BF = jnp.bfloat16
F32 = jnp.float32


def _bf16_round(v):
    u = int(np.float32(v).view(np.uint32))
    u = (u + 0x7FFF + ((u >> 16) & 1)) & 0xFFFF0000
    return float(np.uint32(u).view(np.float32))


SCALE = _bf16_round(DH ** -0.5)
EPS = _bf16_round(1e-5)


def _r(x):
    return x.astype(BF).astype(F32)


def _layernorm(x32):
    m = jnp.mean(x32, axis=-1, keepdims=True)
    c = x32 - m
    v = jnp.mean(c * c, axis=-1, keepdims=True)
    num = _r(x32 - _r(m))
    den = _r(jnp.sqrt(_r(_r(v) + EPS)))
    return (num / den).astype(BF)


def _blocks(rows, cols, phase, max_tiles, block, cuts=()):
    tr, n = cols // 128, rows // 8 * (cols // 128)
    edges = sorted({0, n} | set(range((-phase) % block, n, block)) | {c // 8 * tr for c in cuts})
    out = []
    for lo, hi in zip(edges[:-1], edges[1:]):
        segs = []
        while lo < hi:
            r, c = divmod(lo, tr)
            if c == 0 and hi - lo >= tr and tr <= max_tiles:
                nr = (hi - lo) // tr
                k = -(-nr // (max_tiles // tr))
                segs += [(r + i * nr // k, (i + 1) * nr // k - i * nr // k, 0, tr) for i in range(k)]
                lo += nr * tr
            else:
                nc = min(hi - lo, tr - c)
                k = -(-nc // max_tiles)
                segs += [(r, 1, c + i * nc // k, (i + 1) * nc // k - i * nc // k) for i in range(k)]
                lo += nc
        out.append([(8 * r, 8 * nr, 128 * c, 128 * nc) for r, nr, c, nc in segs])
    return out


def _scatter(blocks, stride):
    return [p for o in range(stride) for blk in blocks[o::stride] for p in blk]


def _window(m, n, tiles, sweep, gstride, cstride, c0, g0):
    groups = [(a, min(n, DH // 8 // m - a), 8 * j, 8) for a in range(0, DH // 8 // m, n) for j in range(m)]
    groups = _scatter([[g] for g in groups], gstride)
    groups = groups[g0:] + groups[:g0]
    bands = W // 128 // tiles
    return [g + ((c * cstride + c0) % bands * tiles * 128, tiles * 128)
            for i in range(0, len(groups), sweep) for c in range(bands) for g in groups[i:i + sweep]]


def _two_threads(tag0, pieces0, tag1, pieces1):
    items = []
    for t, (tag, pieces) in enumerate(((tag0, pieces0), (tag1, pieces1))):
        total, pos = sum(math.prod(p[1::2]) for p in pieces), 0
        for p in pieces:
            items.append((pos / total, t, tag, p))
            pos += math.prod(p[1::2])
    return [(tag, p, t) for _, t, tag, p in sorted(items, key=lambda z: z[:2])]


def _halves(tag, blocks, stride):
    h = max(1, len(blocks) // 2)
    return _two_threads(tag, _scatter(blocks[:h], stride), tag, _scatter(blocks[h:], stride))


def _split(lst, n):
    return [lst[i * len(lst) // n:(i + 1) * len(lst) // n] for i in range(n)]


def make_kernel(R=3, kv=(2, 2, 8), kp=(3, 2, 1, 0, 0), vp=(4, 4, 1, 0, 0), wq=(0, 8, 8, 64), wo=(0, 8, 8, 64), pair=True,
                w13=(0, 8, 8, 32), w2=(0, 8, 8, 16), nq=4, n0=20, DA=384,
                w2ch=(512, 384, 384, 256), w2at=(0, 2, 4), kvp=None, pro=None):
    N2 = len(w2ch)
    w2off = [sum(w2ch[:i]) for i in range(N2)]
    KG, KR = DH // 8 // kv[0], 8 * kv[0]
    kvp = kvp or _two_threads(0, _window(*kv, *kp), 1, _window(*kv, *vp))
    NF = R - 1 + sum(max(0, w2at[c + 1] - w2at[c] - 1) for c in range(2))
    bq = _blocks(D, H * DH, *wq[:3])
    bo = [b for b in _blocks(H * DH, D, *wo[:3], cuts=(8 * NF,)) if b[0][0] >= 8 * NF]
    if pro:
        pro = pro(bq, bo)
    elif pair:
        pro = _two_threads(0, _scatter(bq, wq[3]), 1, _scatter(bo, wo[3]))
    else:
        pro = _halves(0, bq, wq[3]) + _halves(1, bo, wo[3])
    b13 = _blocks(D, F, *w13[:3], cuts=(DA,))
    p13 = [_scatter([b for b in b13 if (b[0][0] >= DA) == c], w13[3]) for c in range(2)]
    w13p = [_two_threads(0, p, 1, p) for p in p13]
    b2 = _blocks(F, D, *w2[:3], cuts=w2off)
    w2p = [_halves(c, [b for b in b2 if w2off[c] <= b[0][0] < w2off[c] + w2ch[c]], w2[3]) for c in range(N2)]
    def kernel(x_hbm, kt_hbm, vt_hbm, wq_hbm, wo_hbm, w1_hbm, w3_hbm, w2_hbm, o_hbm,
               kv_v, wq_v, wo_v, w13_v, w2_v, q_v, x_v, o_v, sem_o):

        def body(sem_f, sem_w, sem_kv, sem_w13, sem_w2):
            def copy(job):
                src, dst, sem, p, _ = job
                idx = tuple(pl.ds(p[i], p[i + 1]) for i in range(0, len(p), 2))
                return pltpu.make_async_copy(src.at[idx], dst.at[idx], sem)

            def issue(jobs):
                for j in jobs:
                    copy(j).start(priority=j[4])

            def wait_all(ref, sem):
                pltpu.make_async_copy(ref, ref, sem).wait()

            def head_jobs(h, slot):
                srcs = [c.at[h, :, :, pl.ds(SK - W, W)] for c in (kt_hbm, vt_hbm)]
                return [(srcs[a], kv_v.at[slot, a], sem_kv.at[slot], p, t) for a, p, t in kvp]

            x_copy = pltpu.make_async_copy(x_hbm, x_v, sem_f.at[0])
            x_copy.start()
            jobs = [(wo_hbm, wo_v, sem_f.at[1 + i], (8 * i, 8, 0, D), (1 + i) % 2) for i in range(NF)]
            fences = [x_copy] + [copy(j) for j in jobs]
            issue(jobs + [((wq_hbm, wo_hbm)[a], (wq_v, wo_v)[a], sem_w, p, t) for a, p, t in pro])
            for h in range(R):
                fences.pop(0).wait()
                jobs = head_jobs(h, h)
                issue(jobs if h < R - 1 else jobs[:n0])
            wait_all(wq_v, sem_w)
            wait_all(wo_v.at[pl.ds(8 * NF, H * DH - 8 * NF)], sem_w)
            x32 = x_v[...].astype(F32)
            lnx = jnp.broadcast_to(_layernorm(x32), (8, D))
            QC = H // nq
            for c, group in enumerate(_split(jobs[n0:], nq)):
                qc = jnp.dot(lnx, wq_v[:, c * QC * DH:(c + 1) * QC * DH], preferred_element_type=F32)
                for j in range(QC):
                    q_v[c * QC + j] = qc[:, j * DH:(j + 1) * DH]
                issue(group)

            def head_compute(h, slot, attn):
                wait_all(kv_v.at[slot], sem_kv.at[slot])
                qh = q_v[h].astype(BF)
                s = jnp.dot(qh, kv_v[slot, 0].reshape(DH, W), preferred_element_type=F32)
                s = _r(_r(s) * SCALE)
                m = jnp.max(s, axis=-1, keepdims=True)
                e = _r(jnp.exp(_r(s - m)))
                l = _r(jnp.sum(e, axis=-1, keepdims=True))
                p = (e / l).astype(BF)
                o = lax.dot_general(p, kv_v[slot, 1].reshape(DH, W), (((1,), (1,)), ((), ())),
                                    preferred_element_type=F32)
                row = h * DH
                if not isinstance(h, int):
                    row = pl.multiple_of(row, DH)
                return attn + jnp.dot(o.astype(BF), wo_v[pl.ds(row, DH), :], preferred_element_type=F32)

            def head(h, attn):
                slot = h % R
                attn = head_compute(h, slot, attn)
                issue(head_jobs(h + R, slot))
                return attn

            attn = lax.fori_loop(0, H - R, head, jnp.zeros((8, D), F32))

            w13j = [[((w1_hbm, w3_hbm)[a], w13_v.at[a], sem_w13.at[c], p, t) for a, p, t in w13p[c]] for c in range(2)]
            w2j = [[(w2_hbm, w2_v, sem_w2.at[c], p, t) for _, p, t in w2p[c]] for c in range(N2)]
            for h, group in zip(range(H - R, H), _split(w13j[0], R - 1) + [w13j[1]]):
                attn = head_compute(h, h % R, attn)
                issue(group)
            hres = _r(x32 + _r(attn))
            lnh = _layernorm(hres)
            gate = up = 0.0
            for c, (r0, r1) in enumerate(((0, DA), (DA, D))):
                wait_all(w13_v.at[:, pl.ds(r0, r1 - r0)], sem_w13.at[c])
                gate = gate + jnp.dot(lnh[:, r0:r1], w13_v[0, r0:r1, :], preferred_element_type=F32)
                up = up + jnp.dot(lnh[:, r0:r1], w13_v[1, r0:r1, :], preferred_element_type=F32)
                for k in range(w2at[c], w2at[c + 1]):
                    if k > w2at[c]:
                        fences.pop(0).wait()
                    issue(w2j[k])
            assert not fences
            gate, up = _r(gate), _r(up)
            hm = (_r(gate * _r(jax.nn.sigmoid(gate))) * up).astype(BF)
            out = None
            for c in range(N2):
                r0, nr = w2off[c], w2ch[c]
                wait_all(w2_v.at[pl.ds(r0, nr)], sem_w2.at[c])
                o_ = jnp.dot(hm[:, r0:r0 + nr], w2_v[r0:r0 + nr, :], preferred_element_type=F32)
                out = o_ if out is None else out + o_
                if w2at[2] + c < N2:
                    issue(w2j[w2at[2] + c])
            res = hres + _r(out)
            o_v[...] = res[0:1, :].astype(o_v.dtype)
            pltpu.make_async_copy(o_v, o_hbm, sem_o).start()

        dma = pltpu.SemaphoreType.DMA
        pl.run_scoped(body, dma((1 + NF,)), dma(()), dma((R,)), dma((2,)), dma((N2,)))
        pltpu.make_async_copy(o_v, o_hbm, sem_o).wait()

    @jax.jit
    def run(A_x, A_k_cache, A_v_cache, A_wq, A_wo, B_x, B_w1, B_w3, B_w2):
        del B_x
        x = A_x.reshape(1, D)
        kt = jnp.swapaxes(A_k_cache.reshape(H, SK, DH), 1, 2).reshape(H, KG, KR, SK)
        vt = jnp.swapaxes(A_v_cache.reshape(H, SK, DH), 1, 2).reshape(H, KG, KR, SK)
        out = pl.pallas_call(
            kernel,
            out_shape=jax.ShapeDtypeStruct((1, D), A_x.dtype),
            in_specs=[pl.BlockSpec(memory_space=pl.ANY)] * 8,
            out_specs=pl.BlockSpec(memory_space=pl.ANY),
            scratch_shapes=[
                pltpu.VMEM((R, 2, KG, KR, W), BF),
                pltpu.VMEM((D, H * DH), BF),
                pltpu.VMEM((H * DH, D), BF),
                pltpu.VMEM((2, D, F), BF),
                pltpu.VMEM((F, D), BF),
                pltpu.VMEM((H, 8, DH), F32),
                pltpu.VMEM((1, D), BF),
                pltpu.VMEM((1, D), BF),
                pltpu.SemaphoreType.DMA(()),
            ],
            compiler_params=pltpu.CompilerParams(vmem_limit_bytes=64 * 1024 * 1024),
        )(x, kt, vt, A_wq, A_wo, B_w1, B_w3, B_w2)
        return out.reshape(1, 1, D)

    return run


pallas_sequential_preLN__sliding_block_cached__glu_gated_swiglu__decode_kernel = make_kernel()
```

```python
import math

import jax
import jax.numpy as jnp
import numpy as np
from jax import lax
import jax.experimental.pallas as pl
import jax.experimental.pallas.tpu as pltpu

H, DH, SK, D, F = 32, 192, 32768, 640, 1536
W = min(4096, max(256, SK // 4))
BF = jnp.bfloat16
F32 = jnp.float32


def _bf16_round(v):
    u = int(np.float32(v).view(np.uint32))
    u = (u + 0x7FFF + ((u >> 16) & 1)) & 0xFFFF0000
    return float(np.uint32(u).view(np.float32))


SCALE = _bf16_round(DH ** -0.5)
EPS = _bf16_round(1e-5)


def _r(x):
    return x.astype(BF).astype(F32)


def _layernorm(x32):
    m = jnp.mean(x32, axis=-1, keepdims=True)
    c = x32 - m
    v = jnp.mean(c * c, axis=-1, keepdims=True)
    num = _r(x32 - _r(m))
    den = _r(jnp.sqrt(_r(_r(v) + EPS)))
    return (num / den).astype(BF)


def _blocks(rows, cols, phase, max_tiles, block, cuts=()):
    tr, n = cols // 128, rows // 8 * (cols // 128)
    edges = sorted({0, n} | set(range((-phase) % block, n, block)) | {c // 8 * tr for c in cuts})
    out = []
    for lo, hi in zip(edges[:-1], edges[1:]):
        segs = []
        while lo < hi:
            r, c = divmod(lo, tr)
            if c == 0 and hi - lo >= tr and tr <= max_tiles:
                nr = (hi - lo) // tr
                k = -(-nr // (max_tiles // tr))
                segs += [(r + i * nr // k, (i + 1) * nr // k - i * nr // k, 0, tr) for i in range(k)]
                lo += nr * tr
            else:
                nc = min(hi - lo, tr - c)
                k = -(-nc // max_tiles)
                segs += [(r, 1, c + i * nc // k, (i + 1) * nc // k - i * nc // k) for i in range(k)]
                lo += nc
        out.append([(8 * r, 8 * nr, 128 * c, 128 * nc) for r, nr, c, nc in segs])
    return out


def _scatter(blocks, stride):
    return [p for o in range(stride) for blk in blocks[o::stride] for p in blk]


def _window(m, runs, tiles, sweep, stride):
    groups = [(a, runs, 8 * j, 8) for a in range(0, DH // 8 // m, runs) for j in range(m)]
    groups = _scatter([[g] for g in groups], stride)
    return [g + (c, tiles * 128)
            for i in range(0, len(groups), sweep) for c in range(0, W, tiles * 128) for g in groups[i:i + sweep]]


def _two_threads(tag0, pieces0, tag1, pieces1):
    items = []
    for t, (tag, pieces) in enumerate(((tag0, pieces0), (tag1, pieces1))):
        total, pos = sum(math.prod(p[1::2]) for p in pieces), 0
        for p in pieces:
            items.append((pos / total, t, tag, p))
            pos += math.prod(p[1::2])
    return [(tag, p, t) for _, t, tag, p in sorted(items, key=lambda z: z[:2])]


def _halves(tag, blocks, stride):
    h = max(1, len(blocks) // 2)
    return _two_threads(tag, _scatter(blocks[:h], stride), tag, _scatter(blocks[h:], stride))


def _split(lst, n):
    return [lst[i * len(lst) // n:(i + 1) * len(lst) // n] for i in range(n)]


def make_kernel(R=2, kv=(2, 2, 8), kp=(3, 2), vp=(4, 4), wq=(0, 8, 8, 64), wo=(0, 8, 8, 64),
                w13=(0, 8, 8, 32), w2=(0, 8, 8, 16), nq=4, DA=384, w2ch=(512, 384, 384, 256), w2at=(0, 2, 4)):
    N2 = len(w2ch)
    NS = R + 1
    w2off = [sum(w2ch[:i]) for i in range(N2)]
    KG, KR = DH // 8 // kv[0], 8 * kv[0]
    kvp = _two_threads(0, _window(*kv, *kp), 1, _window(*kv, *vp))
    FO, FE = R - 1, sum(max(0, w2at[c + 1] - w2at[c] - 1) for c in range(2))
    bq = _blocks(D, H * DH, *wq[:3])
    bo = [b for b in _blocks(H * DH, D, *wo[:3], cuts=(8 * FO,)) if b[0][0] >= 8 * FO]
    pro = _two_threads(0, _scatter(bq, wq[3]), 1, _scatter(bo, wo[3]))
    b13 = _blocks(D, F, *w13[:3], cuts=(DA,))
    p13 = [_scatter([b for b in b13 if (b[0][0] >= DA) == c], w13[3]) for c in range(2)]
    w13p = [_two_threads(0, p, 1, p) for p in p13]
    w2end = w2off[1:] + [F - 8 * FE]
    b2 = _blocks(F, D, *w2[:3], cuts=w2off + w2end)
    w2p = [_halves(c, [b for b in b2 if w2off[c] <= b[0][0] < w2end[c]], w2[3]) for c in range(N2)]

    def kernel(x_hbm, kt_hbm, vt_hbm, wq_hbm, wo_hbm, w1_hbm, w3_hbm, w2_hbm, o_hbm,
               kv_v, wq_v, wo_v, w13_v, w2_v, q_v, x_v, o_v, sem_o):

        def body(sem_f, sem_w, sem_kv, sem_w13, sem_w2):
            def copy(job):
                src, dst, sem, p, _ = job
                idx = tuple(pl.ds(p[i], p[i + 1]) for i in range(0, len(p), 2))
                return pltpu.make_async_copy(src.at[idx], dst.at[idx], sem)

            def issue(jobs):
                for j in jobs:
                    copy(j).start(priority=j[4])

            def wait_all(ref, sem):
                pltpu.make_async_copy(ref, ref, sem).wait()

            def head_jobs(h, slot):
                srcs = [c.at[h, :, :, pl.ds(SK - W, W)] for c in (kt_hbm, vt_hbm)]
                return [(srcs[a], kv_v.at[slot, a], sem_kv.at[2 * slot + a], p, t) for a, p, t in kvp]

            x_copy = pltpu.make_async_copy(x_hbm, x_v, sem_f.at[0])
            x_copy.start()
            jobs = [(wo_hbm, wo_v, 8 * i) for i in range(FO)] + [(w2_hbm, w2_v, F - 8 * (i + 1)) for i in range(FE)]
            jobs = [(src, dst, sem_f.at[1 + i], (r, 8, 0, D), (1 + i) % 2) for i, (src, dst, r) in enumerate(jobs)]
            fences = [x_copy] + [copy(j) for j in jobs]
            issue(jobs + [((wq_hbm, wo_hbm)[a], (wq_v, wo_v)[a], sem_w.at[a], p, t) for a, p, t in pro])
            for h in range(R):
                fences.pop(0).wait()
                issue(head_jobs(h, h))
            wait_all(wq_v, sem_w.at[0])
            wait_all(wo_v.at[pl.ds(8 * FO, H * DH - 8 * FO)], sem_w.at[1])
            x32 = x_v[...].astype(F32)
            lnx = jnp.broadcast_to(_layernorm(x32), (8, D))
            QC = H // nq
            for c in range(nq):
                qc = jnp.dot(lnx, wq_v[:, c * QC * DH:(c + 1) * QC * DH], preferred_element_type=F32)
                for j in range(QC):
                    q_v[c * QC + j] = qc[:, j * DH:(j + 1) * DH]

            def head_compute(h, slot, attn, prefetch=()):
                early, late = _split(prefetch, 2)
                wait_all(kv_v.at[slot, 0], sem_kv.at[2 * slot])
                issue(early)
                qh = q_v[h].astype(BF)
                s = jnp.dot(qh, kv_v[slot, 0].reshape(DH, W), preferred_element_type=F32)
                s = _r(_r(s) * SCALE)
                m = jnp.max(s, axis=-1, keepdims=True)
                e = _r(jnp.exp(_r(s - m)))
                l = _r(jnp.sum(e, axis=-1, keepdims=True))
                p = (e / l).astype(BF)
                wait_all(kv_v.at[slot, 1], sem_kv.at[2 * slot + 1])
                issue(late)
                o = lax.dot_general(p, kv_v[slot, 1].reshape(DH, W), (((1,), (1,)), ((), ())),
                                    preferred_element_type=F32)
                row = h * DH
                if not isinstance(h, int):
                    row = pl.multiple_of(row, DH)
                return attn + jnp.dot(o.astype(BF), wo_v[pl.ds(row, DH), :], preferred_element_type=F32)

            def head(h, attn):
                return head_compute(h, h % NS, attn, head_jobs(h + R, (h + R) % NS))

            attn = lax.fori_loop(0, H - R, head, jnp.zeros((8, D), F32))

            w13j = [[((w1_hbm, w3_hbm)[a], w13_v.at[a], sem_w13.at[c], p, t) for a, p, t in w13p[c]] for c in range(2)]
            w2j = [[(w2_hbm, w2_v, sem_w2.at[c], p, t) for _, p, t in w2p[c]] for c in range(N2)]
            for h, group in zip(range(H - R, H), _split(w13j[0], R - 1) + [w13j[1]]):
                attn = head_compute(h, h % NS, attn, group)
            hres = _r(x32 + _r(attn))
            lnh = _layernorm(hres)
            gate = up = 0.0
            for c, (r0, r1) in enumerate(((0, DA), (DA, D))):
                wait_all(w13_v.at[:, pl.ds(r0, r1 - r0)], sem_w13.at[c])
                gate = gate + jnp.dot(lnh[:, r0:r1], w13_v[0, r0:r1, :], preferred_element_type=F32)
                up = up + jnp.dot(lnh[:, r0:r1], w13_v[1, r0:r1, :], preferred_element_type=F32)
                for k in range(w2at[c], w2at[c + 1]):
                    if k > w2at[c]:
                        fences.pop(0).wait()
                    issue(w2j[k])
            assert not fences and w2at[2] == N2
            gate, up = _r(gate), _r(up)
            hm = (_r(gate * _r(jax.nn.sigmoid(gate))) * up).astype(BF)
            out = None
            for c in range(N2):
                r0, nr = w2off[c], w2ch[c]
                wait_all(w2_v.at[pl.ds(r0, w2end[c] - r0)], sem_w2.at[c])
                o_ = jnp.dot(hm[:, r0:r0 + nr], w2_v[r0:r0 + nr, :], preferred_element_type=F32)
                out = o_ if out is None else out + o_
            res = hres + _r(out)
            o_v[...] = res[0:1, :].astype(o_v.dtype)
            pltpu.make_async_copy(o_v, o_hbm, sem_o).start()

        dma = pltpu.SemaphoreType.DMA
        pl.run_scoped(body, dma((1 + FO + FE,)), dma((2,)), dma((2 * NS,)), dma((2,)), dma((N2,)))
        pltpu.make_async_copy(o_v, o_hbm, sem_o).wait()

    @jax.jit
    def run(A_x, A_k_cache, A_v_cache, A_wq, A_wo, B_x, B_w1, B_w3, B_w2):
        del B_x
        x = A_x.reshape(1, D)
        kt = jnp.swapaxes(A_k_cache.reshape(H, SK, DH), 1, 2).reshape(H, KG, KR, SK)
        vt = jnp.swapaxes(A_v_cache.reshape(H, SK, DH), 1, 2).reshape(H, KG, KR, SK)
        out = pl.pallas_call(
            kernel,
            out_shape=jax.ShapeDtypeStruct((1, D), A_x.dtype),
            in_specs=[pl.BlockSpec(memory_space=pl.ANY)] * 8,
            out_specs=pl.BlockSpec(memory_space=pl.ANY),
            scratch_shapes=[
                pltpu.VMEM((NS, 2, KG, KR, W), BF),
                pltpu.VMEM((D, H * DH), BF),
                pltpu.VMEM((H * DH, D), BF),
                pltpu.VMEM((2, D, F), BF),
                pltpu.VMEM((F, D), BF),
                pltpu.VMEM((H, 8, DH), F32),
                pltpu.VMEM((1, D), BF),
                pltpu.VMEM((1, D), BF),
                pltpu.SemaphoreType.DMA(()),
            ],
            compiler_params=pltpu.CompilerParams(vmem_limit_bytes=64 * 1024 * 1024),
        )(x, kt, vt, A_wq, A_wo, B_w1, B_w3, B_w2)
        return out.reshape(1, 1, D)

    return run


pallas_sequential_preLN__sliding_block_cached__glu_gated_swiglu__decode_kernel = make_kernel()
```

```python
import math

import jax
import jax.numpy as jnp
import numpy as np
from jax import lax
import jax.experimental.pallas as pl
import jax.experimental.pallas.tpu as pltpu

H, DH, SK, D, F = 32, 192, 32768, 640, 1536
W = min(4096, max(256, SK // 4))
BF = jnp.bfloat16
F32 = jnp.float32


def _bf16_round(v):
    u = int(np.float32(v).view(np.uint32))
    u = (u + 0x7FFF + ((u >> 16) & 1)) & 0xFFFF0000
    return float(np.uint32(u).view(np.float32))


SCALE = _bf16_round(DH ** -0.5)
EPS = _bf16_round(1e-5)


def _r(x):
    return x.astype(BF).astype(F32)


def _layernorm(x32):
    m = jnp.mean(x32, axis=-1, keepdims=True)
    c = x32 - m
    v = jnp.mean(c * c, axis=-1, keepdims=True)
    num = _r(x32 - _r(m))
    den = _r(jnp.sqrt(_r(_r(v) + EPS)))
    return (num / den).astype(BF)


def _blocks(rows, cols, phase, max_tiles, block, cuts=()):
    tr, n = cols // 128, rows // 8 * (cols // 128)
    edges = sorted({0, n} | set(range((-phase) % block, n, block)) | {c // 8 * tr for c in cuts})
    out = []
    for lo, hi in zip(edges[:-1], edges[1:]):
        segs = []
        while lo < hi:
            r, c = divmod(lo, tr)
            if c == 0 and hi - lo >= tr and tr <= max_tiles:
                nr = (hi - lo) // tr
                k = -(-nr // (max_tiles // tr))
                segs += [(r + i * nr // k, (i + 1) * nr // k - i * nr // k, 0, tr) for i in range(k)]
                lo += nr * tr
            else:
                nc = min(hi - lo, tr - c)
                k = -(-nc // max_tiles)
                segs += [(r, 1, c + i * nc // k, (i + 1) * nc // k - i * nc // k) for i in range(k)]
                lo += nc
        out.append([(8 * r, 8 * nr, 128 * c, 128 * nc) for r, nr, c, nc in segs])
    return out


def _scatter(blocks, stride):
    return [p for o in range(stride) for blk in blocks[o::stride] for p in blk]


def _window(m, runs, tiles, sweep, stride):
    groups = [(a, runs, 8 * j, 8) for a in range(0, DH // 8 // m, runs) for j in range(m)]
    groups = _scatter([[g] for g in groups], stride)
    return [g + (c, tiles * 128)
            for i in range(0, len(groups), sweep) for c in range(0, W, tiles * 128) for g in groups[i:i + sweep]]


def _two_threads(tag0, pieces0, tag1, pieces1):
    items = []
    for t, (tag, pieces) in enumerate(((tag0, pieces0), (tag1, pieces1))):
        total, pos = sum(math.prod(p[1::2]) for p in pieces), 0
        for p in pieces:
            items.append((pos / total, t, tag, p))
            pos += math.prod(p[1::2])
    return [(tag, p, t) for _, t, tag, p in sorted(items, key=lambda z: z[:2])]


def _halves(tag, blocks, stride):
    h = max(1, len(blocks) // 2)
    return _two_threads(tag, _scatter(blocks[:h], stride), tag, _scatter(blocks[h:], stride))


def _split(lst, n):
    return [lst[i * len(lst) // n:(i + 1) * len(lst) // n] for i in range(n)]


def make_kernel(R=2, kv=(2, 2, 8), kp=(3, 2), vp=(4, 4), wq=(0, 8, 8, 64), wo=(0, 8, 8, 64),
                w13=(0, 8, 8, 32), w2=(0, 8, 8, 16), nq=4, DA=384, w2ch=(512, 384, 384, 256), w2at=(1, 2, 4)):
    N2 = len(w2ch)
    NS = R + 1
    w2off = [sum(w2ch[:i]) for i in range(N2)]
    KG, KR = DH // 8 // kv[0], 8 * kv[0]
    kvp = _two_threads(0, _window(*kv, *kp), 1, _window(*kv, *vp))
    FO, FE = R - 1, w2at[0] + sum(max(0, w2at[c + 1] - w2at[c] - 1) for c in range(2))
    bq = _blocks(D, H * DH, *wq[:3])
    bo = [b for b in _blocks(H * DH, D, *wo[:3], cuts=(8 * FO,)) if b[0][0] >= 8 * FO]
    pro = _two_threads(0, _scatter(bq, wq[3]), 1, _scatter(bo, wo[3]))
    b13 = _blocks(D, F, *w13[:3], cuts=(DA,))
    p13 = [_scatter([b for b in b13 if (b[0][0] >= DA) == c], w13[3]) for c in range(2)]
    w13p = [_two_threads(0, p, 1, p) for p in p13]
    w2end = w2off[1:] + [F - 8 * FE]
    b2 = _blocks(F, D, *w2[:3], cuts=w2off + w2end)
    w2p = [_halves(c, [b for b in b2 if w2off[c] <= b[0][0] < w2end[c]], w2[3]) for c in range(N2)]

    def kernel(x_hbm, kt_hbm, vt_hbm, wq_hbm, wo_hbm, w1_hbm, w3_hbm, w2_hbm, o_hbm,
               kv_v, wq_v, wo_v, w13_v, w2_v, q_v, x_v, o_v, sem_o):

        def body(sem_f, sem_w, sem_kv, sem_w13, sem_w2):
            def copy(job):
                src, dst, sem, p, _ = job
                idx = tuple(pl.ds(p[i], p[i + 1]) for i in range(0, len(p), 2))
                return pltpu.make_async_copy(src.at[idx], dst.at[idx], sem)

            def issue(jobs):
                for j in jobs:
                    copy(j).start(priority=j[4])

            def wait_all(ref, sem):
                pltpu.make_async_copy(ref, ref, sem).wait()

            def head_jobs(h, slot):
                srcs = [c.at[h, :, :, pl.ds(SK - W, W)] for c in (kt_hbm, vt_hbm)]
                return [(srcs[a], kv_v.at[slot, a], sem_kv.at[2 * slot + a], p, t) for a, p, t in kvp]

            x_copy = pltpu.make_async_copy(x_hbm, x_v, sem_f.at[0])
            x_copy.start()
            jobs = [(wo_hbm, wo_v, 8 * i) for i in range(FO)] + [(w2_hbm, w2_v, F - 8 * (i + 1)) for i in range(FE)]
            jobs = [(src, dst, sem_f.at[1 + i], (r, 8, 0, D), (1 + i) % 2) for i, (src, dst, r) in enumerate(jobs)]
            fences = [x_copy] + [copy(j) for j in jobs]
            issue(jobs + [((wq_hbm, wo_hbm)[a], (wq_v, wo_v)[a], sem_w.at[a], p, t) for a, p, t in pro])
            for h in range(R):
                fences.pop(0).wait()
                issue(head_jobs(h, h))
            wait_all(wq_v, sem_w.at[0])
            wait_all(wo_v.at[pl.ds(8 * FO, H * DH - 8 * FO)], sem_w.at[1])
            x32 = x_v[...].astype(F32)
            lnx = jnp.broadcast_to(_layernorm(x32), (8, D))
            QC = H // nq
            for c in range(nq):
                qc = jnp.dot(lnx, wq_v[:, c * QC * DH:(c + 1) * QC * DH], preferred_element_type=F32)
                for j in range(QC):
                    q_v[c * QC + j] = qc[:, j * DH:(j + 1) * DH]

            def head_compute(h, slot, attn, prefetch=()):
                early, late = _split(prefetch, 2)
                wait_all(kv_v.at[slot, 0], sem_kv.at[2 * slot])
                issue(early)
                qh = q_v[h].astype(BF)
                s = jnp.dot(qh, kv_v[slot, 0].reshape(DH, W), preferred_element_type=F32)
                s = _r(_r(s) * SCALE)
                m = jnp.max(s, axis=-1, keepdims=True)
                e = _r(jnp.exp(_r(s - m)))
                l = _r(jnp.sum(e, axis=-1, keepdims=True))
                p = (e / l).astype(BF)
                wait_all(kv_v.at[slot, 1], sem_kv.at[2 * slot + 1])
                issue(late)
                o = lax.dot_general(p, kv_v[slot, 1].reshape(DH, W), (((1,), (1,)), ((), ())),
                                    preferred_element_type=F32)
                row = h * DH
                if not isinstance(h, int):
                    row = pl.multiple_of(row, DH)
                return attn + jnp.dot(o.astype(BF), wo_v[pl.ds(row, DH), :], preferred_element_type=F32)

            def head(h, attn):
                return head_compute(h, h % NS, attn, head_jobs(h + R, (h + R) % NS))

            attn = lax.fori_loop(0, H - R, head, jnp.zeros((8, D), F32))

            w13j = [[((w1_hbm, w3_hbm)[a], w13_v.at[a], sem_w13.at[c], p, t) for a, p, t in w13p[c]] for c in range(2)]
            w2j = [[(w2_hbm, w2_v, sem_w2.at[c], p, t) for _, p, t in w2p[c]] for c in range(N2)]
            for h, group in zip(range(H - R, H), _split(w13j[0], R - 1) + [w13j[1]]):
                attn = head_compute(h, h % NS, attn, group)
            for k in range(w2at[0]):
                fences.pop(0).wait()
                issue(w2j[k])
            hres = _r(x32 + _r(attn))
            lnh = _layernorm(hres)
            gate = up = 0.0
            for c, (r0, r1) in enumerate(((0, DA), (DA, D))):
                wait_all(w13_v.at[:, pl.ds(r0, r1 - r0)], sem_w13.at[c])
                gate = gate + jnp.dot(lnh[:, r0:r1], w13_v[0, r0:r1, :], preferred_element_type=F32)
                up = up + jnp.dot(lnh[:, r0:r1], w13_v[1, r0:r1, :], preferred_element_type=F32)
                for k in range(w2at[c], w2at[c + 1]):
                    if k > w2at[c]:
                        fences.pop(0).wait()
                    issue(w2j[k])
            assert not fences and w2at[2] == N2
            gate, up = _r(gate), _r(up)
            hm = (_r(gate * _r(jax.nn.sigmoid(gate))) * up).astype(BF)
            out = None
            for c in range(N2):
                r0, nr = w2off[c], w2ch[c]
                wait_all(w2_v.at[pl.ds(r0, w2end[c] - r0)], sem_w2.at[c])
                o_ = jnp.dot(hm[:, r0:r0 + nr], w2_v[r0:r0 + nr, :], preferred_element_type=F32)
                out = o_ if out is None else out + o_
            res = hres + _r(out)
            o_v[...] = res[0:1, :].astype(o_v.dtype)
            pltpu.make_async_copy(o_v, o_hbm, sem_o).start()

        dma = pltpu.SemaphoreType.DMA
        pl.run_scoped(body, dma((1 + FO + FE,)), dma((2,)), dma((2 * NS,)), dma((2,)), dma((N2,)))
        pltpu.make_async_copy(o_v, o_hbm, sem_o).wait()

    @jax.jit
    def run(A_x, A_k_cache, A_v_cache, A_wq, A_wo, B_x, B_w1, B_w3, B_w2):
        del B_x
        x = A_x.reshape(1, D)
        kt = jnp.swapaxes(A_k_cache.reshape(H, SK, DH), 1, 2).reshape(H, KG, KR, SK)
        vt = jnp.swapaxes(A_v_cache.reshape(H, SK, DH), 1, 2).reshape(H, KG, KR, SK)
        out = pl.pallas_call(
            kernel,
            out_shape=jax.ShapeDtypeStruct((1, D), A_x.dtype),
            in_specs=[pl.BlockSpec(memory_space=pl.ANY)] * 8,
            out_specs=pl.BlockSpec(memory_space=pl.ANY),
            scratch_shapes=[
                pltpu.VMEM((NS, 2, KG, KR, W), BF),
                pltpu.VMEM((D, H * DH), BF),
                pltpu.VMEM((H * DH, D), BF),
                pltpu.VMEM((2, D, F), BF),
                pltpu.VMEM((F, D), BF),
                pltpu.VMEM((H, 8, DH), F32),
                pltpu.VMEM((1, D), BF),
                pltpu.VMEM((1, D), BF),
                pltpu.SemaphoreType.DMA(()),
            ],
            compiler_params=pltpu.CompilerParams(vmem_limit_bytes=64 * 1024 * 1024),
        )(x, kt, vt, A_wq, A_wo, B_w1, B_w3, B_w2)
        return out.reshape(1, 1, D)

    return run


pallas_sequential_preLN__sliding_block_cached__glu_gated_swiglu__decode_kernel = make_kernel()
```
